```python
import os as _os
_os.environ.setdefault("JAX_PLATFORMS", "cpu")
import jax
import jax.numpy as jnp

def _softmax(x, axis=-1):
    return jax.nn.softmax(x, axis=axis)
def _gelu(x):
    return jax.nn.gelu(x, approximate=True)
def _silu(x):
    return jax.nn.silu(x)
def _sigmoid(x):
    return jax.nn.sigmoid(x)
def _layernorm(x, axis=-1, eps=1e-5):
    m = jnp.mean(x, axis=axis, keepdims=True)
    v = jnp.var(x, axis=axis, keepdims=True)
    return (x - m) / jnp.sqrt(v + eps)
def _scatter_add(tgt, idx, src, axis=0):
    return tgt.at[idx].add(src)
def _segment_sum(src, seg, n):
    return jax.ops.segment_sum(src, seg, n)
class _Rng:
    def __init__(self, key):
        self._k = key
    def _next(self):
        self._k, sub = jax.random.split(self._k)
        return sub
    def normal(self, shape):
        return jax.random.normal(self._next(), shape, dtype=jnp.bfloat16)
    def randint(self, lo, hi, shape):
        return jax.random.randint(self._next(), shape, lo, hi, dtype=jnp.int32)
    def uniform(self, shape, lo=0.0, hi=1.0):
        return jax.random.uniform(self._next(), shape, jnp.bfloat16, lo, hi)
    def permutation(self, n):
        return jax.random.permutation(self._next(), n)


kernel_name = 'gated_mix__gqa_block_cached__dense_activation_squared_relu__decode'

def setup_inputs():
    _rng = _Rng(jax.random.key(int.from_bytes(__import__("os").urandom(4), "little")))
    _w = (lambda a: (lambda t: t.astype(jnp.bfloat16) if jnp.issubdtype(t.dtype, jnp.floating) else t)(jnp.asarray(a)))
    def _A_setup():
        B, Sq, D = 4, 1, 512
        Hq, Hkv, Sk, Dh = 32, 8, 4096, 128
        assert Hq % Hkv == 0, (Hq, Hkv)
        return {
            "x": _w((lambda *s: _rng.normal(s) * 0.05)(B, Sq, D)),
            "k_cache": _w((lambda *s: _rng.normal(s) * 3.2)(B, Hkv, Sk, Dh)),
            "v_cache": _w((lambda *s: _rng.normal(s) * 1.6)(B, Hkv, Sk, Dh)),
            "wq": _w((lambda *s: _rng.normal(s) * 3.2)(D, Hq * Dh) * (D ** -0.5)),
            "wo": _w((lambda *s: _rng.normal(s) * 1.6)(Hq * Dh, D) * ((Hq * Dh) ** -0.5)),
        }
    _A_in = _A_setup()

    def _B_setup():
        B, S, D, F = 4, 1, 512, 1792
        return {
            "x": _w((lambda *s: _rng.normal(s) * 0.05)(B, S, D)),
            "w1": _w((lambda *s: _rng.normal(s) * 0.1)(D, F)),
            "b1": _w((lambda *s: _rng.normal(s) * 0.05)(F)),
            "w2": _w((lambda *s: _rng.normal(s) * 0.05)(F, D)),
            "b2": _w((lambda *s: _rng.normal(s) * 0.05)(D)),
        }
    _B_in = _B_setup()

    return {
        "A_x": _A_in["x"],
        "A_k_cache": _A_in["k_cache"],
        "A_v_cache": _A_in["v_cache"],
        "A_wq": _A_in["wq"],
        "A_wo": _A_in["wo"],
        "B_x": _B_in["x"],
        "B_w1": _B_in["w1"],
        "B_b1": _B_in["b1"],
        "B_w2": _B_in["w2"],
        "B_b2": _B_in["b2"],
        "gate_w": _w((lambda *s: _rng.normal(s) * 0.05)(512) * 16.0),
    }

def reference(A_x, A_k_cache, A_v_cache, A_wq, A_wo, B_x, B_w1, B_b1, B_w2, B_b2, gate_w):
    def _A_ref(x, k_cache, v_cache, wq, wo):
        B, Sq, D = x.shape
        Hq, Dh = 32, 128
        Hkv = k_cache.shape[1]
        rep = Hq // Hkv
        q = (lambda x, *d: x.transpose(*d))((x @ wq).reshape(B, Sq, Hq, Dh), 0, 2, 1, 3)
        k = jnp.repeat(k_cache, rep, axis=1)
        v = jnp.repeat(v_cache, rep, axis=1)
        scores = jnp.einsum("bhqd,bhkd->bhqk", q, k) * (Dh ** -0.5)
        p = _softmax(scores, axis=-1)
        o = jnp.einsum("bhqk,bhkd->bhqd", p, v)
        return (lambda x, *d: x.transpose(*d))(o, 0, 2, 1, 3).reshape(B, Sq, Hq * Dh) @ wo

    def _B_ref(x, w1, b1, w2, b2):
        h = jnp.einsum("bsd,df->bsf", x, w1) + b1
        zero = jnp.zeros_like(h)
        r = jnp.where(h > zero, h, zero)
        h = r * r
        out = jnp.einsum("bsf,fd->bsd", h, w2) + b2
        return out

    x = A_x
    g = _sigmoid((x * gate_w).sum(-1, keepdims=True))
    a = _A_ref(x, A_k_cache, A_v_cache, A_wq, A_wo)
    b = _B_ref(x, B_w1, B_b1, B_w2, B_b2)
    return g * a + (1 - g) * b
```

```python
import functools
import jax
import jax.numpy as jnp
import jax.experimental.pallas as pl
import jax.experimental.pallas.tpu as pltpu

B, D = 4, 512
HQ, HKV, SK, DH = 32, 8, 4096, 128
REP = HQ // HKV
F = 1792
FC = 256
NFC = F // FC


def _kernel(x_ref, k_ref, v_ref, wq_ref, wo_ref, w1_ref, b1_ref, w2_ref, b2_ref, gw_ref,
            out_ref, q_scr, o_scr, acc_scr, ffn_scr):
    h = pl.program_id(0)
    b = pl.program_id(1)

    @pl.when(jnp.logical_and(h == 0, b == 0))
    def _():
        acc_scr[...] = jnp.zeros_like(acc_scr)
        ffn_scr[...] = jnp.zeros_like(ffn_scr)

    @pl.when(b == 0)
    def _():
        x = x_ref[...]
        qa = jnp.dot(x, wq_ref[...], preferred_element_type=jnp.float32)
        for bb in range(B):
            for j in range(REP):
                q_scr[bb, j:j + 1, :] = qa[bb:bb + 1, j * DH:(j + 1) * DH]

    @pl.when(jnp.logical_and(b == 0, h < NFC))
    def _():
        x = x_ref[...]
        hh = jnp.dot(x, w1_ref[...], preferred_element_type=jnp.float32) + b1_ref[...].astype(jnp.float32)
        r = jnp.maximum(hh, 0.0)
        hh = (r * r).astype(jnp.bfloat16)
        ffn_scr[...] += jnp.dot(hh, w2_ref[...], preferred_element_type=jnp.float32)

    q = q_scr[b].astype(jnp.bfloat16)
    k = k_ref[0, 0]
    v = v_ref[0, 0]
    s = jax.lax.dot_general(q, k, (((1,), (1,)), ((), ())), preferred_element_type=jnp.float32)
    s = s * (DH ** -0.5)
    m = jnp.max(s, axis=-1, keepdims=True)
    p = jnp.exp(s - m)
    l = jnp.sum(p, axis=-1, keepdims=True)
    o = jnp.dot(p.astype(jnp.bfloat16), v, preferred_element_type=jnp.float32) / l
    o_scr[b] = o

    @pl.when(b == B - 1)
    def _():
        oa = jnp.concatenate(
            [jnp.concatenate([o_scr[bb, j:j + 1, :] for j in range(REP)], axis=1) for bb in range(B)],
            axis=0)
        acc_scr[...] += jnp.dot(oa.astype(jnp.bfloat16), wo_ref[...],
                                preferred_element_type=jnp.float32)

    @pl.when(jnp.logical_and(h == HKV - 1, b == B - 1))
    def _():
        x = x_ref[...].astype(jnp.float32)
        g = jax.nn.sigmoid(jnp.sum(x * gw_ref[...].astype(jnp.float32), axis=-1, keepdims=True))
        ffn = ffn_scr[...] + b2_ref[...].astype(jnp.float32)
        out_ref[...] = (g * acc_scr[...] + (1.0 - g) * ffn).astype(out_ref.dtype)


@jax.jit
def pallas_gated_mix__gqa_block_cached__dense_activation_squared_relu__decode_kernel(
    A_x, A_k_cache, A_v_cache, A_wq, A_wo, B_x, B_w1, B_b1, B_w2, B_b2, gate_w,
):
    x = A_x.reshape(B, D)
    fidx = lambda h: jnp.minimum(h, NFC - 1)
    out = pl.pallas_call(
        _kernel,
        grid=(HKV, B),
        in_specs=[
            pl.BlockSpec((B, D), lambda h, b: (0, 0)),
            pl.BlockSpec((1, 1, SK, DH), lambda h, b: (b, h, 0, 0)),
            pl.BlockSpec((1, 1, SK, DH), lambda h, b: (b, h, 0, 0)),
            pl.BlockSpec((D, REP * DH), lambda h, b: (0, h)),
            pl.BlockSpec((REP * DH, D), lambda h, b: (h, 0)),
            pl.BlockSpec((D, FC), lambda h, b: (0, fidx(h))),
            pl.BlockSpec((1, FC), lambda h, b: (0, fidx(h))),
            pl.BlockSpec((FC, D), lambda h, b: (fidx(h), 0)),
            pl.BlockSpec((1, D), lambda h, b: (0, 0)),
            pl.BlockSpec((1, D), lambda h, b: (0, 0)),
        ],
        out_specs=pl.BlockSpec((B, D), lambda h, b: (0, 0)),
        out_shape=jax.ShapeDtypeStruct((B, D), A_x.dtype),
        scratch_shapes=[
            pltpu.VMEM((B, REP, DH), jnp.float32),
            pltpu.VMEM((B, REP, DH), jnp.float32),
            pltpu.VMEM((B, D), jnp.float32),
            pltpu.VMEM((B, D), jnp.float32),
        ],
        compiler_params=pltpu.CompilerParams(
            dimension_semantics=("arbitrary", "arbitrary"),
            vmem_limit_bytes=64 * 1024 * 1024,
        ),
    )(x, A_k_cache, A_v_cache, A_wq, A_wo, B_w1, B_b1.reshape(1, F), B_w2, B_b2.reshape(1, D),
      gate_w.reshape(1, D))
    return out.reshape(B, 1, D)
```

```python
import jax
import jax.numpy as jnp
import jax.experimental.pallas as pl
import jax.experimental.pallas.tpu as pltpu

B, D = 4, 512
HQ, HKV, SK, DH = 32, 8, 4096, 128
REP = HQ // HKV
GW = REP * DH
F = 1792
FC = 256
NFC = F // FC

CK = 1024
NB = 4
NCH = SK // CK
GROUP = B * NCH
NITEMS = HKV * GROUP


def _kernel(x_hbm, k_hbm, v_hbm, wq_hbm, wo_hbm, w1_hbm, b1_hbm, w2_hbm, b2_hbm, gw_hbm,
            out_ref,
            x_buf, b1_buf, b2_buf, gw_buf, kbuf, vbuf, wq_buf, wo_buf, w1_buf, w2_buf,
            q_scr, o_scr, acc_scr, ffn_scr, m_scr, l_scr, a_scr,
            sem_small, sem_kv, sem_wq, sem_wo, sem_ffn):

    def small_copies():
        return [
            pltpu.make_async_copy(x_hbm, x_buf, sem_small),
            pltpu.make_async_copy(b1_hbm, b1_buf, sem_small),
            pltpu.make_async_copy(b2_hbm, b2_buf, sem_small),
            pltpu.make_async_copy(gw_hbm, gw_buf, sem_small),
        ]

    def kv_copies(j):
        h = j // GROUP
        r = j % GROUP
        b = r // NCH
        c = r % NCH
        slot = j % NB
        rows = pl.ds(pl.multiple_of(c * CK, CK), CK)
        return (pltpu.make_async_copy(k_hbm.at[b, h, rows], kbuf.at[slot], sem_kv.at[slot]),
                pltpu.make_async_copy(v_hbm.at[b, h, rows], vbuf.at[slot], sem_kv.at[slot]))

    def wq_copy(h):
        return pltpu.make_async_copy(
            wq_hbm.at[:, pl.ds(pl.multiple_of(h * GW, GW), GW)], wq_buf.at[h], sem_wq)

    def wo_copy(h):
        return pltpu.make_async_copy(
            wo_hbm.at[pl.ds(pl.multiple_of(h * GW, GW), GW), :], wo_buf.at[h], sem_wo)

    def w1_copy(f):
        return pltpu.make_async_copy(
            w1_hbm.at[:, pl.ds(pl.multiple_of(f * FC, FC), FC)], w1_buf.at[f], sem_ffn)

    def w2_copy(f):
        return pltpu.make_async_copy(
            w2_hbm.at[pl.ds(pl.multiple_of(f * FC, FC), FC), :], w2_buf.at[f], sem_ffn)

    def issue(j):
        h = j // GROUP
        r = j % GROUP
        static = isinstance(j, int)

        def when(cond, fn):
            if static:
                if cond:
                    fn()
            else:
                pl.when(cond)(fn)

        when(r == 0, lambda: wq_copy(h).start())
        kc, vc = kv_copies(j)
        kc.start()
        vc.start()
        when(r == GROUP - 1, lambda: wo_copy(h).start())

        def start_ffn():
            w1_copy(h).start()
            w2_copy(h).start()
        if static:
            when(r == 1 and h < NFC, start_ffn)
        else:
            when(jnp.logical_and(r == 1, h < NFC), start_ffn)

    sc = small_copies()
    sc[0].start()
    issue(0)
    for cp in sc[1:]:
        cp.start()
    for j in range(1, NB - 1):
        issue(j)

    acc_scr[...] = jnp.zeros_like(acc_scr)
    ffn_scr[...] = jnp.zeros_like(ffn_scr)
    for cp in sc:
        cp.wait()

    def body(i, carry):
        h = i // GROUP
        r = i % GROUP
        b = r // NCH
        c = r % NCH
        slot = i % NB

        @pl.when(i + NB - 1 < NITEMS)
        def _():
            issue(i + NB - 1)

        @pl.when(r == 0)
        def _():
            wq_copy(h).wait()
            qa = jnp.dot(x_buf[...], wq_buf[h], preferred_element_type=jnp.float32)
            for bb in range(B):
                for jj in range(REP):
                    q_scr[bb, jj:jj + 1, :] = qa[bb:bb + 1, jj * DH:(jj + 1) * DH]

        @pl.when(c == 0)
        def _():
            m_scr[...] = jnp.full_like(m_scr, -jnp.inf)
            l_scr[...] = jnp.zeros_like(l_scr)
            a_scr[...] = jnp.zeros_like(a_scr)

        kc, vc = kv_copies(i)
        kc.wait()
        vc.wait()

        q = q_scr[b].astype(jnp.bfloat16)
        s = jax.lax.dot_general(q, kbuf[slot], (((1,), (1,)), ((), ())),
                                preferred_element_type=jnp.float32)
        s = s * (DH ** -0.5)
        m_prev = m_scr[...]
        m_new = jnp.maximum(m_prev, jnp.max(s, axis=-1, keepdims=True))
        alpha = jnp.exp(m_prev - m_new)
        p = jnp.exp(s - m_new)
        l_scr[...] = alpha * l_scr[...] + jnp.sum(p, axis=-1, keepdims=True)
        a_scr[...] = alpha * a_scr[...] + jnp.dot(p.astype(jnp.bfloat16), vbuf[slot],
                                                  preferred_element_type=jnp.float32)
        m_scr[...] = m_new

        @pl.when(c == NCH - 1)
        def _():
            o_scr[b] = a_scr[...] / l_scr[...]

        @pl.when(r == GROUP - 1)
        def _():
            wo_copy(h).wait()
            oa = jnp.concatenate(
                [jnp.concatenate([o_scr[bb, jj:jj + 1, :] for jj in range(REP)], axis=1)
                 for bb in range(B)], axis=0)
            acc_scr[...] += jnp.dot(oa.astype(jnp.bfloat16), wo_buf[h],
                                    preferred_element_type=jnp.float32)

        @pl.when(jnp.logical_and(r == GROUP - NB, h < NFC))
        def _():
            w1_copy(h).wait()
            w2_copy(h).wait()
            b1c = b1_buf[pl.ds(pl.multiple_of(h * FC, FC), FC)].astype(jnp.float32)[None, :]
            hh = jnp.dot(x_buf[...], w1_buf[h], preferred_element_type=jnp.float32) + b1c
            rr = jnp.maximum(hh, 0.0)
            hh = (rr * rr).astype(jnp.bfloat16)
            ffn_scr[...] += jnp.dot(hh, w2_buf[h], preferred_element_type=jnp.float32)

        return carry

    jax.lax.fori_loop(0, NITEMS, body, 0)

    x = x_buf[...].astype(jnp.float32)
    g = jax.nn.sigmoid(jnp.sum(x * gw_buf[...].astype(jnp.float32)[None, :], axis=-1, keepdims=True))
    ffn = ffn_scr[...] + b2_buf[...].astype(jnp.float32)[None, :]
    out_ref[...] = (g * acc_scr[...] + (1.0 - g) * ffn).astype(out_ref.dtype)


@jax.jit
def pallas_gated_mix__gqa_block_cached__dense_activation_squared_relu__decode_kernel(
    A_x: jax.Array,
    A_k_cache: jax.Array,
    A_v_cache: jax.Array,
    A_wq: jax.Array,
    A_wo: jax.Array,
    B_x: jax.Array,
    B_w1: jax.Array,
    B_b1: jax.Array,
    B_w2: jax.Array,
    B_b2: jax.Array,
    gate_w: jax.Array,
):
    bf = jnp.bfloat16
    out = pl.pallas_call(
        _kernel,
        in_specs=[pl.BlockSpec(memory_space=pl.ANY)] * 10,
        out_specs=pl.BlockSpec(memory_space=pltpu.VMEM),
        out_shape=jax.ShapeDtypeStruct((B, D), A_x.dtype),
        scratch_shapes=[
            pltpu.VMEM((B, D), bf),
            pltpu.VMEM((F,), bf),
            pltpu.VMEM((D,), bf),
            pltpu.VMEM((D,), bf),
            pltpu.VMEM((NB, CK, DH), bf),
            pltpu.VMEM((NB, CK, DH), bf),
            pltpu.VMEM((HKV, D, GW), bf),
            pltpu.VMEM((HKV, GW, D), bf),
            pltpu.VMEM((NFC, D, FC), bf),
            pltpu.VMEM((NFC, FC, D), bf),
            pltpu.VMEM((B, REP, DH), jnp.float32),
            pltpu.VMEM((B, REP, DH), jnp.float32),
            pltpu.VMEM((B, D), jnp.float32),
            pltpu.VMEM((B, D), jnp.float32),
            pltpu.VMEM((REP, 1), jnp.float32),
            pltpu.VMEM((REP, 1), jnp.float32),
            pltpu.VMEM((REP, DH), jnp.float32),
            pltpu.SemaphoreType.DMA(()),
            pltpu.SemaphoreType.DMA((NB,)),
            pltpu.SemaphoreType.DMA(()),
            pltpu.SemaphoreType.DMA(()),
            pltpu.SemaphoreType.DMA(()),
        ],
        compiler_params=pltpu.CompilerParams(vmem_limit_bytes=64 * 1024 * 1024),
    )(A_x.reshape(B, D), A_k_cache, A_v_cache, A_wq, A_wo, B_w1, B_b1, B_w2, B_b2, gate_w)
    return out.reshape(B, 1, D)
```
